```python
import os as _os
_os.environ.setdefault("JAX_PLATFORMS", "cpu")
import jax
import jax.numpy as jnp

def _softmax(x, axis=-1):
    return jax.nn.softmax(x, axis=axis)
def _gelu(x):
    return jax.nn.gelu(x, approximate=True)
def _silu(x):
    return jax.nn.silu(x)
def _sigmoid(x):
    return jax.nn.sigmoid(x)
def _layernorm(x, axis=-1, eps=1e-5):
    m = jnp.mean(x, axis=axis, keepdims=True)
    v = jnp.var(x, axis=axis, keepdims=True)
    return (x - m) / jnp.sqrt(v + eps)
def _scatter_add(tgt, idx, src, axis=0):
    return tgt.at[idx].add(src)
def _segment_sum(src, seg, n):
    return jax.ops.segment_sum(src, seg, n)
class _Rng:
    def __init__(self, key):
        self._k = key
    def _next(self):
        self._k, sub = jax.random.split(self._k)
        return sub
    def normal(self, shape):
        return jax.random.normal(self._next(), shape, dtype=jnp.bfloat16)
    def randint(self, lo, hi, shape):
        return jax.random.randint(self._next(), shape, lo, hi, dtype=jnp.int32)
    def uniform(self, shape, lo=0.0, hi=1.0):
        return jax.random.uniform(self._next(), shape, jnp.bfloat16, lo, hi)
    def permutation(self, n):
        return jax.random.permutation(self._next(), n)


kernel_name = 'standalone__dcn_v2_cross__recsys'

def setup_inputs():
    _rng = _Rng(jax.random.key(int.from_bytes(__import__("os").urandom(4), "little")))
    _w = (lambda a: (lambda t: t.astype(jnp.bfloat16) if jnp.issubdtype(t.dtype, jnp.floating) else t)(jnp.asarray(a)))
    B, F, D, L = 4096, 26, 128, 6
    Din = min(F * D, 1024)
    return {
        "x0": _w((lambda *s: _rng.normal(s) * 0.05)(B, Din)),
        "ws": _w((lambda *s: _rng.normal(s) * 0.05)(L, Din, Din)),
        "bs": _w((lambda *s: _rng.normal(s) * 0.05)(L, Din)),
    }

def reference(x0, ws, bs):
    x = x0
    for l in range(ws.shape[0]):
        x = x0 * (x @ ws[l] + bs[l]) + x
    return x
```

```python
import functools

import jax
import jax.numpy as jnp
import jax.experimental.pallas as pl
import jax.experimental.pallas.tpu as pltpu


def _kernel(x0_ref, ws_ref, bs_ref, o_ref, *, num_layers):
    x0 = x0_ref[...].astype(jnp.float32)
    x = x0
    for l in range(num_layers):
        y = jnp.dot(x.astype(jnp.bfloat16), ws_ref[l],
                    preferred_element_type=jnp.float32)
        y = y + bs_ref[l:l + 1, :].astype(jnp.float32)
        x = x0 * y + x
    o_ref[...] = x.astype(o_ref.dtype)


@jax.jit
def pallas_standalone__dcn_v2_cross__recsys_kernel(
    x0: jax.Array,
    ws: jax.Array,
    bs: jax.Array,
):
    B, D = x0.shape
    L = ws.shape[0]
    tm = 512
    return pl.pallas_call(
        functools.partial(_kernel, num_layers=L),
        grid=(B // tm,),
        in_specs=[
            pl.BlockSpec((tm, D), lambda i: (i, 0)),
            pl.BlockSpec((L, D, D), lambda i: (0, 0, 0)),
            pl.BlockSpec((L, D), lambda i: (0, 0)),
        ],
        out_specs=pl.BlockSpec((tm, D), lambda i: (i, 0)),
        out_shape=jax.ShapeDtypeStruct((B, D), x0.dtype),
        compiler_params=pltpu.CompilerParams(
            dimension_semantics=("arbitrary",),
            vmem_limit_bytes=100 * 1024 * 1024,
        ),
    )(x0, ws, bs)
```

```python
import functools

import jax
import jax.numpy as jnp
from jax import lax
import jax.experimental.pallas as pl
import jax.experimental.pallas.tpu as pltpu

bf = jnp.bfloat16
f32 = jnp.float32
u32 = jnp.uint32

SA = (
    (((0, 0), 1), ((1, 1), 1)),
    (((1, 0), 1), ((1, 1), 1)),
    (((0, 0), 1),),
    (((1, 1), 1),),
    (((0, 0), 1), ((0, 1), 1)),
    (((1, 0), 1), ((0, 0), -1)),
    (((0, 1), 1), ((1, 1), -1)),
)
SB = (
    (((0, 0), 1), ((1, 1), 1)),
    (((0, 0), 1),),
    (((0, 1), 1), ((1, 1), -1)),
    (((1, 0), 1), ((0, 0), -1)),
    (((1, 1), 1),),
    (((0, 0), 1), ((0, 1), 1)),
    (((1, 0), 1), ((1, 1), 1)),
)
ORDER = (2, 4, 1, 3, 0, 6, 5)


def _signed_sum(terms):
    terms = sorted(terms, key=lambda t: -t[1])
    acc, s0 = terms[0]
    assert s0 == 1
    for v, s in terms[1:]:
        acc = acc + v if s > 0 else acc - v
    return acc


def _two_level_terms(tab, p, s):
    return [((2 * I + i, 2 * J + j), s1 * s2)
            for (I, J), s1 in tab[p] for (i, j), s2 in tab[s]]


def _combine_step(s, m, ld, st, emit):
    if s == 2:
        st(0, m)
    elif s == 4:
        st(1, m)
        emit((0, 1), m + ld(0))
    elif s == 1:
        st(2, m)
    elif s == 3:
        st(3, m)
        emit((1, 0), m + ld(2))
    elif s == 0:
        st(4, m + ld(3) - ld(1))
        st(5, m + ld(0) - ld(2))
    elif s == 6:
        emit((0, 0), m + ld(4))
    elif s == 5:
        emit((1, 1), m + ld(5))


def _prep_piece(wr_l, wc_ref, p, s, row0, nrows, q, tie):
    v = _signed_sum([(wr_l[pl.ds(i * q + row0, nrows), j * q:(j + 1) * q].astype(f32), sg)
                     for (i, j), sg in _two_level_terms(SB, p, s)])
    pv = pltpu.bitcast(v.astype(bf), u32)
    flag, tv = tie
    pv = jnp.where(flag, tv, pv)
    h0 = pl.multiple_of(row0 // 2, nrows // 2)
    wc_ref[p * 7 + s, pl.ds(h0, nrows // 2), :] = pv


def _prep_full(wr_l, wc_ref, q, rows=16):
    for g in range(q // rows):
        row0 = g * rows
        blk = {(i, j): wr_l[i * q + row0:i * q + row0 + rows, j * q:(j + 1) * q].astype(f32)
               for i in range(4) for j in range(4)}
        for p in range(7):
            lvl1 = {(i, j): _signed_sum([(blk[(2 * I + i, 2 * J + j)], s1) for (I, J), s1 in SB[p]])
                    for i in range(2) for j in range(2)}
            for s in range(7):
                v = _signed_sum([(lvl1[ij], s2) for ij, s2 in SB[s]])
                wc_ref[p * 7 + s, row0 // 2:(row0 + rows) // 2, :] = pltpu.bitcast(v.astype(bf), u32)


def _make_tie(m, nrows, q):
    r = m.shape[0]
    ng = nrows // 16
    nc = q // 128
    step = r // (ng * nc)
    rows = []
    for a in range(ng):
        rows.append(jnp.concatenate(
            [m[(a * nc + n) * step:(a * nc + n) * step + 8, n * 128:(n + 1) * 128]
             for n in range(nc)], axis=1))
    return pltpu.bitcast(jnp.concatenate(rows, axis=0), u32)


def _tile_layer(src, x0t, dst, wc_ref, bias_load, MS, PS, r, q, prep):
    def sl(i, j):
        return (slice(i * r, (i + 1) * r), slice(j * q, (j + 1) * q))

    def src_load(i, j):
        return src[sl(i, j)].astype(f32)

    for p in ORDER:
        for s in ORDER:
            terms = _two_level_terms(SA, p, s)
            if len(terms) == 1:
                lhs = src[sl(*terms[0][0])].astype(bf)
            else:
                lhs = _signed_sum([(src_load(i, j), sg) for (i, j), sg in terms]).astype(bf)
            rhs = pltpu.bitcast(wc_ref[p * 7 + s], bf)
            m = jnp.dot(lhs, rhs, preferred_element_type=f32)
            if prep is not None:
                prep(p, s, m)
            if p in (2, 3) and s in (2, 3):
                gj = 2 * (1 if p == 2 else 0) + (1 if s == 2 else 0)
                m = m + bias_load(gj)

            def emit2(ij, v, p=p):
                i, j = ij
                slot = 2 * i + j

                def emit1(IJ, y):
                    gi, gj = 2 * IJ[0] + i, 2 * IJ[1] + j
                    z = x0t[sl(gi, gj)].astype(f32)
                    dst[sl(gi, gj)] = (z * y + src_load(gi, gj)).astype(dst.dtype)

                def st1(kk, vv):
                    PS[kk, slot] = vv

                _combine_step(p, v, lambda kk: PS[kk, slot], st1, emit1)

            def st2(kk, vv):
                MS[kk] = vv

            _combine_step(s, m, lambda kk: MS[kk], st2, emit2)


def _kernel(x0_hbm, ws_hbm, bs_ref, out_hbm, X0, XA, XB, WR, WCA, WCB, OUT, BF, MS, PS, ZS,
            sem_x, sem_w, sem_c, sem_o, *, B, D, L, tm):
    nt = B // tm
    r = tm // 4
    q = D // 4
    pr = q // nt

    def x_copy(t):
        return pltpu.make_async_copy(x0_hbm.at[pl.ds(t * tm, tm)], X0.at[pl.ds(t * tm, tm)], sem_x.at[t])

    def w_copy(l):
        return pltpu.make_async_copy(ws_hbm.at[l], WR.at[l], sem_w.at[l])

    def w1_chunk(t, i):
        rows = pl.ds(i * q + t * pr, pr)
        return pltpu.make_async_copy(ws_hbm.at[1, rows], WR.at[1, rows], sem_c.at[t * 4 + i])

    def o_copy(t):
        return pltpu.make_async_copy(OUT.at[pl.ds(t * tm, tm)], out_hbm.at[pl.ds(t * tm, tm)], sem_o.at[t])

    w_copy(0).start()
    BF[...] = bs_ref[...].astype(f32)
    ZS[0] = 0
    w_copy(0).wait()
    x_copy(0).start()
    for i in range(4):
        w1_chunk(0, i).start()
    _prep_full(WR.at[0], WCA, q)

    def tile(ref, t):
        return ref.at[pl.ds(pl.multiple_of(t * tm, tm), tm)]

    def run_layer(l, src, dst, wc, wc_next, first=False, last=False):
        def body(t, c):
            if first:
                x_copy(t).wait()
                for i in range(4):
                    w1_chunk(t, i).wait()

                @pl.when(t + 1 < nt)
                def _():
                    x_copy(t + 1).start()
                    for i in range(4):
                        w1_chunk(t + 1, i).start()

                @pl.when(t + 1 == nt)
                def _():
                    w_copy(2).start()
            prep = None
            if not last:
                wr_l = WR.at[l + 1]
                row0 = pl.multiple_of(t * pr, pr)
                flag = ZS[0] != 0
                prep = lambda p, s, m: _prep_piece(wr_l, wc_next, p, s, row0, pr, q,
                                                   (flag, _make_tie(m, pr, q)))
            if isinstance(l, int):
                bias_load = lambda j: BF[l:l + 1, j * q:(j + 1) * q]
            else:
                bias_load = lambda j: BF[pl.ds(l, 1), j * q:(j + 1) * q]
            _tile_layer(tile(src, t), tile(X0, t), tile(dst, t), wc, bias_load, MS, PS, r, q, prep)
            if last:
                o_copy(t).start()
            return c
        lax.fori_loop(0, nt, body, 0)

    run_layer(0, X0, XA, WCA, WCB, first=True)

    def pair(i, c):
        l = 1 + 2 * i
        w_copy(l + 1).wait()
        w_copy(l + 2).start()
        run_layer(l, XA, XB, WCB, WCA)
        w_copy(l + 2).wait()

        @pl.when(l + 3 < L)
        def _():
            w_copy(l + 3).start()
        run_layer(l + 1, XB, XA, WCA, WCB)
        return c
    lax.fori_loop(0, (L - 2) // 2, pair, 0)
    run_layer(L - 1, XA, OUT, WCB, None, last=True)
    for t in range(nt):
        o_copy(t).wait()


@jax.jit
def pallas_standalone__dcn_v2_cross__recsys_kernel(
    x0: jax.Array,
    ws: jax.Array,
    bs: jax.Array,
):
    B, D = x0.shape
    L = ws.shape[0]
    tm = 1024
    q = D // 4
    nt = B // tm
    r = tm // 4
    return pl.pallas_call(
        functools.partial(_kernel, B=B, D=D, L=L, tm=tm),
        in_specs=[
            pl.BlockSpec(memory_space=pl.ANY),
            pl.BlockSpec(memory_space=pl.ANY),
            pl.BlockSpec(memory_space=pltpu.VMEM),
        ],
        out_specs=pl.BlockSpec(memory_space=pl.ANY),
        out_shape=jax.ShapeDtypeStruct((B, D), x0.dtype),
        scratch_shapes=[
            pltpu.VMEM((B, D), bf),
            pltpu.VMEM((B, D), f32),
            pltpu.VMEM((B, D), f32),
            pltpu.VMEM((L, D, D), bf),
            pltpu.VMEM((49, q // 2, q), u32),
            pltpu.VMEM((49, q // 2, q), u32),
            pltpu.VMEM((B, D), bf),
            pltpu.VMEM((L, D), f32),
            pltpu.VMEM((6, r, q), f32),
            pltpu.VMEM((6, 4, r, q), f32),
            pltpu.SMEM((1,), jnp.int32),
            pltpu.SemaphoreType.DMA((nt,)),
            pltpu.SemaphoreType.DMA((L,)),
            pltpu.SemaphoreType.DMA((4 * nt,)),
            pltpu.SemaphoreType.DMA((nt,)),
        ],
        compiler_params=pltpu.CompilerParams(
            vmem_limit_bytes=120 * 1024 * 1024,
        ),
    )(x0, ws, bs)
```

```python
import functools

import jax
import jax.numpy as jnp
from jax import lax
import jax.experimental.pallas as pl
import jax.experimental.pallas.tpu as pltpu

bf = jnp.bfloat16
f32 = jnp.float32

_SA = (
    (((0, 0), 1), ((1, 1), 1)),
    (((1, 0), 1), ((1, 1), 1)),
    (((0, 0), 1),),
    (((1, 1), 1),),
    (((0, 0), 1), ((0, 1), 1)),
    (((1, 0), 1), ((0, 0), -1)),
    (((0, 1), 1), ((1, 1), -1)),
)
_SB = (
    (((0, 0), 1), ((1, 1), 1)),
    (((0, 0), 1),),
    (((0, 1), 1), ((1, 1), -1)),
    (((1, 0), 1), ((0, 0), -1)),
    (((1, 1), 1),),
    (((0, 0), 1), ((0, 1), 1)),
    (((1, 0), 1), ((1, 1), 1)),
)
_ORDER = (2, 4, 1, 3, 0, 6, 5)


def _signed_sum(terms):
    terms = sorted(terms, key=lambda t: -t[1])
    acc, s0 = terms[0]
    assert s0 == 1
    for v, s in terms[1:]:
        acc = acc + v if s > 0 else acc - v
    return acc


def _two_level_terms(tab, p, s):
    return [((2 * I + i, 2 * J + j), s1 * s2)
            for (I, J), s1 in tab[p] for (i, j), s2 in tab[s]]


def _combine_step(s, m, ld, st, emit):
    if s == 2:
        st(0, m)
    elif s == 4:
        st(1, m)
        emit((0, 1), m + ld(0))
    elif s == 1:
        st(2, m)
    elif s == 3:
        st(3, m)
        emit((1, 0), m + ld(2))
    elif s == 0:
        st(4, m + ld(3) - ld(1))
        st(5, m + ld(0) - ld(2))
    elif s == 6:
        emit((0, 0), m + ld(4))
    elif s == 5:
        emit((1, 1), m + ld(5))


def _prep_piece(wr_l, wc_ref, p, s, row0, nrows, q, never, m):
    nc = q // 128
    ng = nrows // 16
    rg = m.shape[0] // 8
    for a in range(ng):
        v = _signed_sum([(wr_l[pl.ds(i * q + row0 + a * 16, 16), j * q:(j + 1) * q].astype(f32), sg)
                         for (i, j), sg in _two_level_terms(_SB, p, s)])
        for n in range(nc):
            g = ((a * nc + n) * rg) // (ng * nc)
            cols = slice(n * 128, (n + 1) * 128)
            top = jnp.where(never, m[g * 8:g * 8 + 8, cols], v[0:8, cols])
            vv = jnp.concatenate([top, v[8:16, cols]], axis=0)
            wc_ref[p * 7 + s, n, pl.ds(row0 + a * 16, 16), :] = vv.astype(bf)


def _prep_rows(wr_l, wc_ref, q, r0, nrows, rows=16):
    for g in range(nrows // rows):
        row0 = r0 + g * rows
        blk = {(i, j): wr_l[i * q + row0:i * q + row0 + rows, j * q:(j + 1) * q].astype(f32)
               for i in range(4) for j in range(4)}
        for p in range(7):
            lvl1 = {(i, j): _signed_sum([(blk[(2 * I + i, 2 * J + j)], s1) for (I, J), s1 in _SB[p]])
                    for i in range(2) for j in range(2)}
            for s in range(7):
                v = _signed_sum([(lvl1[ij], s2) for ij, s2 in _SB[s]])
                for n in range(q // 128):
                    wc_ref[p * 7 + s, n, row0:row0 + rows, :] = v[:, n * 128:(n + 1) * 128].astype(bf)


def _tile_layer(src, x0t, dst, wc_ref, bias_load, MS, PS, r, q, prep, done, swap):
    def sl(i, j):
        i = i ^ swap
        return (slice(i * r, (i + 1) * r), slice(j * q, (j + 1) * q))

    def src_load(i, j):
        return src[sl(i, j)].astype(f32)

    for p in _ORDER:
        for s in _ORDER:
            terms = _two_level_terms(_SA, p, s)
            if len(terms) == 1:
                lhs = src[sl(*terms[0][0])].astype(bf)
            else:
                lhs = _signed_sum([(src_load(i, j), sg) for (i, j), sg in terms]).astype(bf)
            rhs = jnp.concatenate([wc_ref[p * 7 + s, n] for n in range(q // 128)], axis=1)
            m = jnp.dot(lhs, rhs, preferred_element_type=f32)
            if prep is not None:
                prep(p, s, m)
            if p in (2, 3) and s in (2, 3):
                gj = 2 * (1 if p == 2 else 0) + (1 if s == 2 else 0)
                m = m + bias_load(gj)

            def emit2(ij, v, p=p):
                i, j = ij
                slot = 2 * i + j

                def emit1(IJ, y):
                    gi, gj = 2 * IJ[0] + i, 2 * IJ[1] + j
                    z = x0t[sl(gi, gj)].astype(f32)
                    dst[sl(gi, gj)] = (z * y + src_load(gi, gj)).astype(dst.dtype)
                    if done is not None:
                        done(IJ, ij)

                def st1(kk, vv):
                    PS[kk, slot, 0:r] = vv

                _combine_step(p, v, lambda kk: PS[kk, slot, 0:r], st1, emit1)

            def st2(kk, vv):
                MS[kk, 0:r] = vv

            _combine_step(s, m, lambda kk: MS[kk, 0:r], st2, emit2)


def _kernel(x0_hbm, ws_hbm, bs_hbm, out_hbm, X0, XA, XB, WR, WCA, WCB, OUT, BS, BF, MS, PS, ZS,
            sem_x, sem_w, sem_c, sem_w0, sem_b, sem_o, *, B, D, L, tm, heads, G):
    nt = B // tm
    r = tm // 4
    q = D // 4
    pr = q // nt
    gr = q // G
    nh = len(heads)
    hoff = [sum(heads[:k]) for k in range(nh)]
    sw0, swab, swba, swl = 0, 1, 2, 3

    def x_rows(r0, n, k):
        return pltpu.make_async_copy(x0_hbm.at[pl.ds(r0, n)], X0.at[pl.ds(r0, n)], sem_x.at[k])

    def xh(k):
        return x_rows(hoff[k], heads[k], k)

    def xt(t):
        return x_rows(t * tm, tm, nh - 1 + t)

    def w_copy(l):
        return pltpu.make_async_copy(ws_hbm.at[l], WR.at[l], sem_w.at[l - 2])

    def w_rows(l, sem, k, r0, n):
        rows = pl.ds(r0, n)
        return pltpu.make_async_copy(ws_hbm.at[l, rows], WR.at[l, rows], sem.at[k])

    def b_copy():
        return pltpu.make_async_copy(bs_hbm, BS, sem_b.at[0])

    def w0c(g, i):
        return w_rows(0, sem_w0, g * 4 + i, i * q + g * gr, gr)

    def w1a(i):
        return w_rows(1, sem_c, i, i * q, pr)

    def w1b(i):
        return w_rows(1, sem_c, 4 + i, i * q + pr, q - pr)

    def o_big(t, IJ, k):
        rows = pl.ds(t * tm + (IJ[0] ^ (swl >> 1)) * 2 * r, 2 * r)
        cols = pl.ds(IJ[1] * 2 * q, 2 * q)
        return pltpu.make_async_copy(OUT.at[rows, cols], out_hbm.at[rows, cols], sem_o.at[t * 7 + k])

    def o_small(t, ij, k):
        rows = pl.ds(t * tm + ((2 + ij[0]) ^ swl) * r, r)
        cols = pl.ds(2 * q + ij[1] * q, q)
        return pltpu.make_async_copy(OUT.at[rows, cols], out_hbm.at[rows, cols], sem_o.at[t * 7 + k])

    big = {(0, 1): 0, (1, 0): 1, (0, 0): 2}
    small = {(0, 1): 3, (1, 0): 4, (0, 0): 5, (1, 1): 6}

    later = [
        [xh(k) for k in range(nh)],
        [w1a(i) for i in range(4)],
        [xt(1)],
        [w1b(i) for i in range(4)],
        [xt(t) for t in range(2, nt)],
        [w_copy(l) for l in range(2, L)],
    ]
    b_copy().start()
    for g in range(G):
        for i in range(4):
            w0c(g, i).start()
    ZS[0] = 0
    for g in range(G):
        for i in range(4):
            w0c(g, i).wait()
            if later:
                for c in later.pop(0):
                    c.start()
        if g == G - 1:
            b_copy().wait()
            BF[...] = BS[...].astype(f32)
        _prep_rows(WR.at[0], WCA, q, g * gr, gr)

    def tile(ref, t):
        return ref.at[pl.ds(pl.multiple_of(t * tm, tm), tm)]

    def mk_prep(l, wc_next, row0):
        wr_l = WR.at[l + 1]
        never = ZS[0] != 0
        return lambda p, s, m: _prep_piece(wr_l, wc_next, p, s, row0, pr, q, never, m)

    for k in range(nh):
        xh(k).wait()
        prep = None
        if k == nh - 1:
            for i in range(4):
                w1a(i).wait()
            prep = mk_prep(0, WCB, 0)
        rows = slice(hoff[k], hoff[k] + heads[k])
        _tile_layer(X0.at[rows], X0.at[rows], XA.at[rows], WCA,
                    lambda j: BF[0:1, j * q:(j + 1) * q], MS, PS, heads[k] // 4, q, prep, None, sw0)
    for i in range(4):
        w1b(i).wait()

    def run_layer(l, src, dst, wc, wc_next, swap, first=False, last=False):
        def body(t, c):
            if first:
                xt(t).wait()
            prep = None
            done = None
            if not last:
                prep = mk_prep(l, wc_next, pl.multiple_of(t * pr, pr))
            else:
                def done(IJ, ij):
                    if IJ == (1, 1):
                        o_small(t, ij, small[ij]).start()
                    elif ij == (1, 1):
                        o_big(t, IJ, big[IJ]).start()
            if isinstance(l, int):
                bias_load = lambda j: BF[l:l + 1, j * q:(j + 1) * q]
            else:
                bias_load = lambda j: BF[pl.ds(l, 1), j * q:(j + 1) * q]
            _tile_layer(tile(src, t), tile(X0, t), tile(dst, t), wc, bias_load, MS, PS, r, q,
                        prep, done, swap)
            return c
        lax.fori_loop(1 if first else 0, nt, body, 0)

    run_layer(0, X0, XA, WCA, WCB, sw0, first=True)

    def pair(i, c):
        l = 1 + 2 * i
        w_copy(l + 1).wait()
        run_layer(l, XA, XB, WCB, WCA, swab)
        w_copy(l + 2).wait()
        run_layer(l + 1, XB, XA, WCA, WCB, swba)
        return c
    lax.fori_loop(0, (L - 2) // 2, pair, 0)
    run_layer(L - 1, XA, OUT, WCB, None, swl, last=True)
    for t in range(nt):
        for IJ, k in big.items():
            o_big(t, IJ, k).wait()
        for ij, k in small.items():
            o_small(t, ij, k).wait()


@jax.jit
def pallas_standalone__dcn_v2_cross__recsys_kernel(
    x0: jax.Array,
    ws: jax.Array,
    bs: jax.Array,
):
    B, D = x0.shape
    L = ws.shape[0]
    tm = 1024
    heads = (320, 704)
    G = 4
    assert B % tm == 0 and D % 512 == 0 and L % 2 == 0 and L >= 4
    q = D // 4
    nt = B // tm
    r = tm // 4
    return pl.pallas_call(
        functools.partial(_kernel, B=B, D=D, L=L, tm=tm, heads=heads, G=G),
        in_specs=[pl.BlockSpec(memory_space=pl.ANY)] * 3,
        out_specs=pl.BlockSpec(memory_space=pl.ANY),
        out_shape=jax.ShapeDtypeStruct((B, D), x0.dtype),
        scratch_shapes=[
            pltpu.VMEM((B, D), bf),
            pltpu.VMEM((B, D), f32),
            pltpu.VMEM((B, D), f32),
            pltpu.VMEM((L, D, D), bf),
            pltpu.VMEM((49, q // 128, q, 128), bf),
            pltpu.VMEM((49, q // 128, q, 128), bf),
            pltpu.VMEM((B, D), bf),
            pltpu.VMEM((L, D), bf),
            pltpu.VMEM((L, D), f32),
            pltpu.VMEM((6, r, q), f32),
            pltpu.VMEM((6, 4, r, q), f32),
            pltpu.SMEM((1,), jnp.int32),
            pltpu.SemaphoreType.DMA((nt - 1 + len(heads),)),
            pltpu.SemaphoreType.DMA((L - 2,)),
            pltpu.SemaphoreType.DMA((8,)),
            pltpu.SemaphoreType.DMA((4 * G,)),
            pltpu.SemaphoreType.DMA((1,)),
            pltpu.SemaphoreType.DMA((7 * nt,)),
        ],
        compiler_params=pltpu.CompilerParams(
            vmem_limit_bytes=120 * 1024 * 1024,
        ),
    )(x0, ws, bs)
```

```python
import functools

import jax
import jax.numpy as jnp
from jax import lax
import jax.experimental.pallas as pl
import jax.experimental.pallas.tpu as pltpu

bf = jnp.bfloat16
f32 = jnp.float32

_SA = (
    (((0, 0), 1), ((1, 1), 1)),
    (((1, 0), 1), ((1, 1), 1)),
    (((0, 0), 1),),
    (((1, 1), 1),),
    (((0, 0), 1), ((0, 1), 1)),
    (((1, 0), 1), ((0, 0), -1)),
    (((0, 1), 1), ((1, 1), -1)),
)
_SB = (
    (((0, 0), 1), ((1, 1), 1)),
    (((0, 0), 1),),
    (((0, 1), 1), ((1, 1), -1)),
    (((1, 0), 1), ((0, 0), -1)),
    (((1, 1), 1),),
    (((0, 0), 1), ((0, 1), 1)),
    (((1, 0), 1), ((1, 1), 1)),
)
_ORDER = (2, 4, 1, 3, 0, 6, 5)
_ALL = (0, 1, 2, 3, 4, 5, 6)
_TOP = (1, 5)
_REST = (2, 4, 3, 0, 6)


def _signed_sum(terms):
    terms = sorted(terms, key=lambda t: -t[1])
    acc, s0 = terms[0]
    assert s0 == 1
    for v, s in terms[1:]:
        acc = acc + v if s > 0 else acc - v
    return acc


def _two_level_terms(tab, p, s):
    return [((2 * I + i, 2 * J + j), s1 * s2)
            for (I, J), s1 in tab[p] for (i, j), s2 in tab[s]]


def _combine_step(s, m, ld, st, emit):
    if s == 2:
        st(0, m)
    elif s == 4:
        st(1, m)
        emit((0, 1), m + ld(0))
    elif s == 1:
        st(2, m)
    elif s == 3:
        st(3, m)
        emit((1, 0), m + ld(2))
    elif s == 0:
        st(4, m + ld(3) - ld(1))
        st(5, m + ld(0) - ld(2))
    elif s == 6:
        emit((0, 0), m + ld(4))
    elif s == 5:
        emit((1, 1), m + ld(5))


def _store_tied(wc_ref, k, n, row0, v, never, anchor):
    top = jnp.where(never, anchor, v[0:8])
    wc_ref[k, n, pl.ds(row0, 16), :] = jnp.concatenate([top, v[8:16]], axis=0).astype(bf)


def _prep_piece(wr_l, wc_ref, p, s, row0, nrows, q, never, m):
    nc = q // 128
    ng = nrows // 16
    rg = m.shape[0] // 8
    for a in range(ng):
        v = _signed_sum([(wr_l[pl.ds(i * q + row0 + a * 16, 16), j * q:(j + 1) * q].astype(f32), sg)
                         for (i, j), sg in _two_level_terms(_SB, p, s)])
        for n in range(nc):
            g = ((a * nc + n) * rg) // (ng * nc)
            cols = slice(n * 128, (n + 1) * 128)
            _store_tied(wc_ref, p * 7 + s, n, row0 + a * 16, v[:, cols], never, m[g * 8:g * 8 + 8, cols])


def _prep_jobs(wr_l, wc_ref, q, jobs, groups, never, m):
    nrg, ncg = m.shape[0] // 8, m.shape[1] // 128
    order = [(g, c) for cp in range(ncg // 2) for g in range(nrg) for c in (2 * cp, 2 * cp + 1)]
    total = len(groups) * sum(len(ss) for _, ss in jobs) * (q // 128)
    cnt = 0
    for g in groups:
        row0 = g * 16
        for p, ss in jobs:
            need = sorted({ij for s in ss for ij, _ in _SB[s]})
            lvl1 = {
                (i, j): _signed_sum([
                    (wr_l[(2 * I + i) * q + row0:(2 * I + i) * q + row0 + 16,
                          (2 * J + j) * q:(2 * J + j + 1) * q].astype(f32), s1)
                    for (I, J), s1 in _SB[p]])
                for (i, j) in need}
            for s in ss:
                v = _signed_sum([(lvl1[ij], s2) for ij, s2 in _SB[s]])
                for n in range(q // 128):
                    tg, tc = order[(cnt * len(order)) // total]
                    cnt += 1
                    _store_tied(wc_ref, p * 7 + s, n, row0, v[:, n * 128:(n + 1) * 128], never,
                                m[tg * 8:tg * 8 + 8, tc * 128:(tc + 1) * 128])


def _tile_layer(src, x0t, dst, wc_ref, bias_load, MS, PS, r, q, prep, done, swap):
    def sl(i, j):
        i = i ^ swap
        return (slice(i * r, (i + 1) * r), slice(j * q, (j + 1) * q))

    def src_load(i, j):
        return src[sl(i, j)].astype(f32)

    for p in _ORDER:
        for s in _ORDER:
            terms = _two_level_terms(_SA, p, s)
            if len(terms) == 1:
                lhs = src[sl(*terms[0][0])].astype(bf)
            else:
                lhs = _signed_sum([(src_load(i, j), sg) for (i, j), sg in terms]).astype(bf)
            rhs = jnp.concatenate([wc_ref[p * 7 + s, n] for n in range(q // 128)], axis=1)
            m = jnp.dot(lhs, rhs, preferred_element_type=f32)
            if prep is not None:
                prep(p, s, m)
            if p in (2, 3) and s in (2, 3):
                gj = 2 * (1 if p == 2 else 0) + (1 if s == 2 else 0)
                m = m + bias_load(gj)

            def emit2(ij, v, p=p):
                i, j = ij
                slot = 2 * i + j

                def emit1(IJ, y):
                    gi, gj = 2 * IJ[0] + i, 2 * IJ[1] + j
                    z = x0t[sl(gi, gj)].astype(f32)
                    dst[sl(gi, gj)] = (z * y + src_load(gi, gj)).astype(dst.dtype)
                    if done is not None:
                        done(IJ, ij)

                def st1(kk, vv):
                    PS[kk, slot, 0:r] = vv

                _combine_step(p, v, lambda kk: PS[kk, slot, 0:r], st1, emit1)

            def st2(kk, vv):
                MS[kk, 0:r] = vv

            _combine_step(s, m, lambda kk: MS[kk, 0:r], st2, emit2)


def _kernel(x0_hbm, ws_hbm, bs_hbm, out_hbm, X0, XA, XB, WR, WCA, WCB, OUT, BS, BF, MS, PS, ZS,
            sem_x, sem_w, sem_c, sem_w0, sem_b, sem_o, *, B, D, L, tm, R, h1):
    nt = B // tm
    r = tm // 4
    q = D // 4
    pr = q // nt
    t0r = R + h1
    tm0 = (B - t0r) // nt
    sw0, swab, swba, swl = 0, 1, 2, 3
    all_groups = list(range(q // 16))

    def xc(k):
        rows, cols = pl.ds(0, R), pl.ds(k * q, q)
        return pltpu.make_async_copy(x0_hbm.at[rows, cols], X0.at[rows, cols], sem_x.at[k])

    def x_rows(r0, n, k):
        return pltpu.make_async_copy(x0_hbm.at[pl.ds(r0, n)], X0.at[pl.ds(r0, n)], sem_x.at[k])

    def xh():
        return x_rows(R, h1, 4)

    def xt(t):
        return x_rows(t0r + t * tm0, tm0, 5 + t)

    def w_copy(l):
        return pltpu.make_async_copy(ws_hbm.at[l], WR.at[l], sem_w.at[l - 2])

    def w_rows(l, sem, k, r0, n):
        rows = pl.ds(r0, n)
        return pltpu.make_async_copy(ws_hbm.at[l, rows], WR.at[l, rows], sem.at[k])

    def b_copy():
        return pltpu.make_async_copy(bs_hbm, BS, sem_b.at[0])

    def wk(k):
        return w_rows(0, sem_w0, k, k * q, q)

    def w1a(i):
        return w_rows(1, sem_c, i, i * q, pr)

    def w1b(i):
        return w_rows(1, sem_c, 4 + i, i * q + pr, q - pr)

    def o_big(t, IJ, k):
        rows = pl.ds(t * tm + (IJ[0] ^ (swl >> 1)) * 2 * r, 2 * r)
        cols = pl.ds(IJ[1] * 2 * q, 2 * q)
        return pltpu.make_async_copy(OUT.at[rows, cols], out_hbm.at[rows, cols], sem_o.at[t * 7 + k])

    def o_small(t, ij, k):
        rows = pl.ds(t * tm + ((2 + ij[0]) ^ swl) * r, r)
        cols = pl.ds(2 * q + ij[1] * q, q)
        return pltpu.make_async_copy(OUT.at[rows, cols], out_hbm.at[rows, cols], sem_o.at[t * 7 + k])

    big = {(0, 1): 0, (1, 0): 1, (0, 0): 2}
    small = {(0, 1): 3, (1, 0): 4, (0, 0): 5, (1, 1): 6}

    later = [
        [xc(2), wk(2)],
        [xc(3), wk(3)],
        [xh()],
        [xt(0)],
        [w1a(i) for i in range(4)],
        [xt(1)],
        [w1b(i) for i in range(4)],
        [xt(t) for t in range(2, nt)],
        [w_copy(l) for l in range(2, L)],
    ]

    def wait_then_issue(c):
        c.wait()
        if later:
            for d in later.pop(0):
                d.start()

    b_copy().start()
    for k in range(2):
        xc(k).start()
        wk(k).start()
    ZS[0] = 0
    never = ZS[0] != 0
    wait_then_issue(b_copy())
    BF[...] = BS[...].astype(f32)

    acc = XB.at[0:R]
    w0 = WR.at[0]
    for k in range(4):
        wait_then_issue(xc(k))
        wait_then_issue(wk(k))
        m = jnp.dot(X0[0:R, k * q:(k + 1) * q], WR[0, k * q:(k + 1) * q, :],
                    preferred_element_type=f32)
        if k == 1:
            _prep_jobs(w0, WCA, q, [(p, _ALL) for p in _TOP], all_groups, never, m)
        elif k == 2:
            _prep_jobs(w0, WCA, q, [(p, _TOP) for p in _REST], all_groups, never, m)
        elif k == 3:
            _prep_jobs(w0, WCA, q, [(p, _REST) for p in _REST[:3]], all_groups, never, m)
        if k == 0:
            acc[...] = m + BF[0:1, :]
        elif k < 3:
            acc[...] = m + acc[...]
        else:
            z = X0[0:R, :].astype(f32)
            XA[0:R, :] = z * (m + acc[...]) + z
    assert not later

    def bias0(j):
        return BF[0:1, j * q:(j + 1) * q]

    def mk_prep(l, wc_next, row0):
        wr_l = WR.at[l + 1]
        nv = ZS[0] != 0
        return lambda p, s, m: _prep_piece(wr_l, wc_next, p, s, row0, pr, q, nv, m)

    nlate = 8
    seq = [(p, s) for p in _ORDER for s in _ORDER][:nlate]

    def prep_late(p, s, m):
        if (p, s) in seq:
            k = seq.index((p, s))
            gs = [g for g in all_groups if (g * nlate) // len(all_groups) == k]
            _prep_jobs(w0, WCA, q, [(pp, _REST) for pp in _REST[3:]], gs, never, m)

    xh().wait()
    rows = slice(R, t0r)
    _tile_layer(X0.at[rows], X0.at[rows], XA.at[rows], WCA, bias0, MS, PS, h1 // 4, q,
                prep_late, None, sw0)
    for i in range(4):
        w1a(i).wait()

    def body0(t, c):
        xt(t).wait()

        @pl.when(t == 1)
        def _():
            for i in range(4):
                w1b(i).wait()
        rows = pl.ds(pl.multiple_of(t0r + t * tm0, 64), tm0)
        _tile_layer(X0.at[rows], X0.at[rows], XA.at[rows], WCA, bias0, MS, PS, tm0 // 4, q,
                    mk_prep(0, WCB, pl.multiple_of(t * pr, pr)), None, sw0)
        return c
    lax.fori_loop(0, nt, body0, 0)

    def tile(ref, t):
        return ref.at[pl.ds(pl.multiple_of(t * tm, tm), tm)]

    def run_layer(l, src, dst, wc, wc_next, swap):
        def body(t, c):
            prep = None
            done = None
            if wc_next is not None:
                prep = mk_prep(l, wc_next, pl.multiple_of(t * pr, pr))
            else:
                def done(IJ, ij):
                    if IJ == (1, 1):
                        o_small(t, ij, small[ij]).start()
                    elif ij == (1, 1):
                        o_big(t, IJ, big[IJ]).start()
            if isinstance(l, int):
                bias_load = lambda j: BF[l:l + 1, j * q:(j + 1) * q]
            else:
                bias_load = lambda j: BF[pl.ds(l, 1), j * q:(j + 1) * q]
            _tile_layer(tile(src, t), tile(X0, t), tile(dst, t), wc, bias_load, MS, PS, r, q,
                        prep, done, swap)
            return c
        lax.fori_loop(0, nt, body, 0)

    def pair(i, c):
        l = 1 + 2 * i
        w_copy(l + 1).wait()
        run_layer(l, XA, XB, WCB, WCA, swab)
        w_copy(l + 2).wait()
        run_layer(l + 1, XB, XA, WCA, WCB, swba)
        return c
    lax.fori_loop(0, (L - 2) // 2, pair, 0)
    run_layer(L - 1, XA, OUT, WCB, None, swl)
    for t in range(nt):
        for IJ, k in big.items():
            o_big(t, IJ, k).wait()
        for ij, k in small.items():
            o_small(t, ij, k).wait()


@jax.jit
def pallas_standalone__dcn_v2_cross__recsys_kernel(
    x0: jax.Array,
    ws: jax.Array,
    bs: jax.Array,
):
    B, D = x0.shape
    L = ws.shape[0]
    tm, R, h1 = 1024, 320, 448
    q = D // 4
    nt = B // tm
    r = tm // 4
    assert B % tm == 0 and D % 1024 == 0 and L % 2 == 0 and L >= 4 and nt >= 2
    assert (B - R - h1) % (64 * nt) == 0 and (q // nt) % 16 == 0
    return pl.pallas_call(
        functools.partial(_kernel, B=B, D=D, L=L, tm=tm, R=R, h1=h1),
        in_specs=[pl.BlockSpec(memory_space=pl.ANY)] * 3,
        out_specs=pl.BlockSpec(memory_space=pl.ANY),
        out_shape=jax.ShapeDtypeStruct((B, D), x0.dtype),
        scratch_shapes=[
            pltpu.VMEM((B, D), bf),
            pltpu.VMEM((B, D), f32),
            pltpu.VMEM((B, D), f32),
            pltpu.VMEM((L, D, D), bf),
            pltpu.VMEM((49, q // 128, q, 128), bf),
            pltpu.VMEM((49, q // 128, q, 128), bf),
            pltpu.VMEM((B, D), bf),
            pltpu.VMEM((L, D), bf),
            pltpu.VMEM((L, D), f32),
            pltpu.VMEM((6, r, q), f32),
            pltpu.VMEM((6, 4, r, q), f32),
            pltpu.SMEM((1,), jnp.int32),
            pltpu.SemaphoreType.DMA((5 + nt,)),
            pltpu.SemaphoreType.DMA((L - 2,)),
            pltpu.SemaphoreType.DMA((8,)),
            pltpu.SemaphoreType.DMA((4,)),
            pltpu.SemaphoreType.DMA((1,)),
            pltpu.SemaphoreType.DMA((7 * nt,)),
        ],
        compiler_params=pltpu.CompilerParams(
            vmem_limit_bytes=120 * 1024 * 1024,
        ),
    )(x0, ws, bs)
```

```python
import functools

import jax
import jax.numpy as jnp
from jax import lax
import jax.experimental.pallas as pl
import jax.experimental.pallas.tpu as pltpu

bf = jnp.bfloat16
f32 = jnp.float32

_SA = (
    (((0, 0), 1), ((1, 1), 1)),
    (((1, 0), 1), ((1, 1), 1)),
    (((0, 0), 1),),
    (((1, 1), 1),),
    (((0, 0), 1), ((0, 1), 1)),
    (((1, 0), 1), ((0, 0), -1)),
    (((0, 1), 1), ((1, 1), -1)),
)
_SB = (
    (((0, 0), 1), ((1, 1), 1)),
    (((0, 0), 1),),
    (((0, 1), 1), ((1, 1), -1)),
    (((1, 0), 1), ((0, 0), -1)),
    (((1, 1), 1),),
    (((0, 0), 1), ((0, 1), 1)),
    (((1, 0), 1), ((1, 1), 1)),
)
_ORDER = (2, 4, 1, 3, 0, 6, 5)
_ALL = (0, 1, 2, 3, 4, 5, 6)
_TOP = (1, 5)
_REST = (2, 4, 3, 0, 6)
_TAU = 1.5
_STAT_SLOTS = (0, 1, 2, 3, 5, 6, 14, 16)


def _signed_sum(terms):
    terms = sorted(terms, key=lambda t: -t[1])
    acc, s0 = terms[0]
    assert s0 == 1
    for v, s in terms[1:]:
        acc = acc + v if s > 0 else acc - v
    return acc


def _two_level_terms(tab, p, s):
    return [((2 * I + i, 2 * J + j), s1 * s2)
            for (I, J), s1 in tab[p] for (i, j), s2 in tab[s]]


def _combine_step(s, m, ld, st, emit):
    if s == 2:
        st(0, m)
    elif s == 4:
        st(1, m)
        emit((0, 1), m + ld(0))
    elif s == 1:
        st(2, m)
    elif s == 3:
        st(3, m)
        emit((1, 0), m + ld(2))
    elif s == 0:
        st(4, m + ld(3) - ld(1))
        st(5, m + ld(0) - ld(2))
    elif s == 6:
        emit((0, 0), m + ld(4))
    elif s == 5:
        emit((1, 1), m + ld(5))


def _store_tied(wc_ref, k, n, row0, v, never, anchor):
    top = jnp.where(never, anchor, v[0:8])
    wc_ref[k, n, pl.ds(row0, 16), :] = jnp.concatenate([top, v[8:16]], axis=0).astype(bf)


def _prep_piece(wr_l, wc_ref, p, s, row0, nrows, q, never, m):
    nc = q // 128
    ng = nrows // 16
    rg = m.shape[0] // 8
    for a in range(ng):
        v = _signed_sum([(wr_l[pl.ds(i * q + row0 + a * 16, 16), j * q:(j + 1) * q].astype(f32), sg)
                         for (i, j), sg in _two_level_terms(_SB, p, s)])
        for n in range(nc):
            g = ((a * nc + n) * rg) // (ng * nc)
            cols = slice(n * 128, (n + 1) * 128)
            _store_tied(wc_ref, p * 7 + s, n, row0 + a * 16, v[:, cols], never, m[g * 8:g * 8 + 8, cols])


def _prep_jobs(wr_l, wc_ref, q, jobs, groups, never, m):
    nrg, ncg = m.shape[0] // 8, m.shape[1] // 128
    order = [(g, c) for cp in range(ncg // 2) for g in range(nrg) for c in (2 * cp, 2 * cp + 1)]
    total = len(groups) * sum(len(ss) for _, ss in jobs) * (q // 128)
    cnt = 0
    for g in groups:
        row0 = g * 16
        for p, ss in jobs:
            need = sorted({ij for s in ss for ij, _ in _SB[s]})
            lvl1 = {
                (i, j): _signed_sum([
                    (wr_l[(2 * I + i) * q + row0:(2 * I + i) * q + row0 + 16,
                          (2 * J + j) * q:(2 * J + j + 1) * q].astype(f32), s1)
                    for (I, J), s1 in _SB[p]])
                for (i, j) in need}
            for s in ss:
                v = _signed_sum([(lvl1[ij], s2) for ij, s2 in _SB[s]])
                for n in range(q // 128):
                    tg, tc = order[(cnt * len(order)) // total]
                    cnt += 1
                    _store_tied(wc_ref, p * 7 + s, n, row0, v[:, n * 128:(n + 1) * 128], never,
                                m[tg * 8:tg * 8 + 8, tc * 128:(tc + 1) * 128])


def _scale_stats(WR, CS, RX, RN, l, row0, never, m):
    ncg = WR.shape[2] // 128
    rg = m.shape[0] // 8

    def anchor(idx):
        g = (idx * rg) // 16
        return m[g * 8:g * 8 + 8, (idx % 2) * 128:(idx % 2) * 128 + 128]

    for c in range(ncg // 2):
        a = jnp.abs(WR[l, pl.ds(row0, 32), c * 256:(c + 1) * 256].astype(f32))
        part = (a[0:8] + a[8:16]) + (a[16:24] + a[24:32])
        for h in range(2):
            cols = slice(c * 256 + h * 128, c * 256 + (h + 1) * 128)
            v = jnp.where(never, anchor(2 * c + h), part[:, h * 128:(h + 1) * 128])
            CS[l, :, cols] = CS[l, :, cols] + v
    for g in range(4):
        a = jnp.abs(WR[l, pl.ds(row0 + (g // 2) * 16, 16), :].astype(f32))
        a = a[(g % 2) * 8:(g % 2) * 8 + 8]
        part = a[:, 0:128]
        for c in range(1, ncg):
            part = part + a[:, c * 128:(c + 1) * 128]
        part = jnp.where(never, anchor(8 + 2 * g), part)
        rs = jnp.broadcast_to(jnp.sum(part, axis=1, keepdims=True), (8, 128))
        RX[l] = jnp.maximum(RX[l], rs)
        RN[l] = jnp.minimum(RN[l], rs)


def _tile_layer(src, x0t, dst, wc_ref, bias_load, MS, PS, r, q, side, done, swap):
    def sl(i, j):
        i = i ^ swap
        return (slice(i * r, (i + 1) * r), slice(j * q, (j + 1) * q))

    def src_load(i, j):
        return src[sl(i, j)].astype(f32)

    for p in _ORDER:
        for s in _ORDER:
            terms = _two_level_terms(_SA, p, s)
            if len(terms) == 1:
                lhs = src[sl(*terms[0][0])].astype(bf)
            else:
                lhs = _signed_sum([(src_load(i, j), sg) for (i, j), sg in terms]).astype(bf)
            rhs = jnp.concatenate([wc_ref[p * 7 + s, n] for n in range(q // 128)], axis=1)
            m = jnp.dot(lhs, rhs, preferred_element_type=f32)
            side(p, s, m)
            if p in (2, 3) and s in (2, 3):
                gj = 2 * (1 if p == 2 else 0) + (1 if s == 2 else 0)
                m = m + bias_load(gj)

            def emit2(ij, v, p=p):
                i, j = ij
                slot = 2 * i + j

                def emit1(IJ, y):
                    gi, gj = 2 * IJ[0] + i, 2 * IJ[1] + j
                    z = x0t[sl(gi, gj)].astype(f32)
                    dst[sl(gi, gj)] = (z * y + src_load(gi, gj)).astype(dst.dtype)
                    if done is not None:
                        done(IJ, ij)

                def st1(kk, vv):
                    PS[kk, slot, 0:r] = vv

                _combine_step(p, v, lambda kk: PS[kk, slot, 0:r], st1, emit1)

            def st2(kk, vv):
                MS[kk, 0:r] = vv

            _combine_step(s, m, lambda kk: MS[kk, 0:r], st2, emit2)


def _kernel(x0_hbm, ws_hbm, bs_hbm, out_hbm, X0, XA, XB, WR, WCA, WCB, OUT, BS, BF, MS, PS,
            CS, RX, RN, ZS, sems, *, B, D, L, tm, R, h1):
    nt = B // tm
    r = tm // 4
    q = D // 4
    pr = q // nt
    t0r = R + h1
    tm0 = (B - t0r) // nt
    sw0, swab, swba, swl = 0, 1, 2, 3
    all_groups = list(range(q // 16))

    def xc(k):
        rows, cols = pl.ds(0, R), pl.ds(k * q, q)
        return pltpu.make_async_copy(x0_hbm.at[rows, cols], X0.at[rows, cols], sems.at[k])

    def x_rows(r0, n, k):
        return pltpu.make_async_copy(x0_hbm.at[pl.ds(r0, n)], X0.at[pl.ds(r0, n)], sems.at[k])

    def w_rows(l, r0, n, k):
        rows = pl.ds(r0, n)
        return pltpu.make_async_copy(ws_hbm.at[l, rows], WR.at[l, rows], sems.at[k])

    head = [[xc(k), w_rows(0, k * q, q, k)] for k in range(4)]
    head[0].insert(0, pltpu.make_async_copy(bs_hbm, BS, sems.at[0]))
    g_h = [x_rows(R, h1, 0)]
    g_t = [[x_rows(t0r + t * tm0, tm0, (1 + t) % 4)] for t in range(nt)]
    g_t[0] += [w_rows(1, i * q, pr, 1) for i in range(4)]
    g_t[1] += [w_rows(1, i * q + pr, q - pr, 2) for i in range(4)]
    g_w = [pltpu.make_async_copy(ws_hbm.at[l], WR.at[l], sems.at[1]) for l in range(2, L)]

    def o_big(t, IJ):
        rows = pl.ds(t * tm + (IJ[0] ^ (swl >> 1)) * 2 * r, 2 * r)
        cols = pl.ds(IJ[1] * 2 * q, 2 * q)
        return pltpu.make_async_copy(OUT.at[rows, cols], out_hbm.at[rows, cols], sems.at[0])

    def o_small(t, ij):
        rows = pl.ds(t * tm + ((2 + ij[0]) ^ swl) * r, r)
        cols = pl.ds(2 * q + ij[1] * q, q)
        return pltpu.make_async_copy(OUT.at[rows, cols], out_hbm.at[rows, cols], sems.at[0])

    def start(group):
        for c in group:
            c.start()

    def wait(group):
        for c in group:
            c.wait()

    def mk_prep(l, wc_next, row0):
        wr_l = WR.at[l + 1]
        nv = ZS[0] != 0
        return lambda p, s, m: _prep_piece(wr_l, wc_next, p, s, row0, pr, q, nv, m)

    def bias0(j):
        return BF[0:1, j * q:(j + 1) * q]

    def layer0():
        start(head[0])
        start(head[1])
        ZS[0] = 0
        never = ZS[0] != 0
        CS[...] = jnp.zeros(CS.shape, f32)
        RX[...] = jnp.zeros(RX.shape, f32)
        RN[...] = jnp.full(RN.shape, jnp.inf, f32)

        acc = XB.at[0:R]
        w0 = WR.at[0]
        for k in range(4):
            if k == 0:
                head[0][0].wait()
                start(head[2])
                head[0][1].wait()
                start(head[3])
                head[0][2].wait()
                start(g_h)
                BF[...] = BS[...].astype(f32)
            else:
                wait(head[k])
                start(g_t[k - 1])
            m = jnp.dot(X0[0:R, k * q:(k + 1) * q], WR[0, k * q:(k + 1) * q, :],
                        preferred_element_type=f32)
            if k == 1:
                _prep_jobs(w0, WCA, q, [(p, _ALL) for p in _TOP], all_groups, never, m)
            elif k == 2:
                _prep_jobs(w0, WCA, q, [(p, _TOP) for p in _REST], all_groups, never, m)
            elif k == 3:
                _prep_jobs(w0, WCA, q, [(p, _REST) for p in _REST[:3]], all_groups, never, m)
            if k == 0:
                acc[...] = m + BF[0:1, :]
            elif k < 3:
                acc[...] = m + acc[...]
            else:
                z = X0[0:R, :].astype(f32)
                XA[0:R, :] = z * (m + acc[...]) + z

        seq = [(p, s) for p in _ORDER for s in _ORDER][:len(all_groups)]

        def prep_late(p, s, m):
            if (p, s) in seq:
                _prep_jobs(w0, WCA, q, [(pp, _REST) for pp in _REST[3:]], [seq.index((p, s))],
                           never, m)

        wait(g_h)
        start(g_t[3])
        rows = slice(R, t0r)
        _tile_layer(X0.at[rows], X0.at[rows], XA.at[rows], WCA, bias0, MS, PS, h1 // 4, q,
                    prep_late, None, sw0)
        wait(g_t[0])
        start(g_w)

        def body0(t, c):
            for tt in range(1, nt):
                @pl.when(t == tt)
                def _():
                    wait(g_t[tt])
            rows = pl.ds(pl.multiple_of(t0r + t * tm0, 64), tm0)
            _tile_layer(X0.at[rows], X0.at[rows], XA.at[rows], WCA, bias0, MS, PS, tm0 // 4, q,
                        mk_prep(0, WCB, pl.multiple_of(t * pr, pr)), None, sw0)
            return c
        lax.fori_loop(0, nt, body0, 0)
        wait(g_w)

    def tile(ref, t):
        return ref.at[pl.ds(pl.multiple_of(t * tm, tm), tm)]

    def run_layer(l, src, dst, wc, wc_next, swap):
        def body(t, c):
            done = None
            nv = ZS[0] != 0
            row_base = pl.multiple_of(t * (D // nt), D // nt)
            if wc_next is not None:
                prep_w = mk_prep(l, wc_next, pl.multiple_of(t * pr, pr))

                def side(p, s, m):
                    prep_w(p, s, m)
                    k = _ORDER.index(p) * 7 + _ORDER.index(s)
                    if k in _STAT_SLOTS:
                        _scale_stats(WR, CS, RX, RN, l + 1, row_base + 32 * _STAT_SLOTS.index(k), nv, m)
            else:
                def side(p, s, m):
                    k = _ORDER.index(p) * 7 + _ORDER.index(s)
                    if k < 16:
                        _scale_stats(WR, CS, RX, RN, k // 8, row_base + 32 * (k % 8), nv, m)

                def done(IJ, ij):
                    if IJ != (1, 1) and ij != (1, 1):
                        return
                    for tt in range(nt):
                        @pl.when(t == tt)
                        def _():
                            if IJ == (1, 1):
                                o_small(tt, ij).start()
                            else:
                                o_big(tt, IJ).start()
            if isinstance(l, int):
                bias_load = lambda j: BF[l:l + 1, j * q:(j + 1) * q]
            else:
                bias_load = lambda j: BF[pl.ds(l, 1), j * q:(j + 1) * q]
            _tile_layer(tile(src, t), tile(X0, t), tile(dst, t), wc, bias_load, MS, PS, r, q,
                        side, done, swap)
            return c
        lax.fori_loop(0, nt, body, 0)

    def two_layers(i, c):
        l = 2 * i

        @pl.when(i == 0)
        def _():
            layer0()

        @pl.when(i > 0)
        def _():
            run_layer(l, XB, XA, WCA, WCB, swba)

        @pl.when(i < L // 2 - 1)
        def _():
            run_layer(l + 1, XA, XB, WCB, WCA, swab)

        @pl.when(i == L // 2 - 1)
        def _():
            run_layer(L - 1, XA, OUT, WCB, None, swl)
        return c
    lax.fori_loop(0, L // 2, two_layers, 0)

    nbad = jnp.zeros((1, 1), f32)
    for l in range(L):
        col = jnp.sum(CS[l], axis=0, keepdims=True)
        cx = jnp.max(col, axis=1, keepdims=True)
        cn = jnp.min(col, axis=1, keepdims=True)
        rx = jnp.max(RX[l][:, 0:1], axis=0, keepdims=True)
        rn = jnp.min(RN[l][:, 0:1], axis=0, keepdims=True)
        nbad = nbad + jnp.where(cx <= _TAU * cn, 0.0, 1.0) + jnp.where(rx <= _TAU * rn, 0.0, 1.0)
    bad = nbad[0, 0] > 0.0

    pltpu.make_async_copy(OUT, out_hbm, sems.at[0]).wait()

    @pl.when(bad)
    def _():
        tf = 128
        xs = XA.at[0:tf]

        def tile_body(t, c):
            rows = pl.ds(pl.multiple_of(t * tf, tf), tf)
            xs[...] = X0[rows, :].astype(f32)

            def layer_body(l, c2):
                x = xs[...]
                y = jnp.dot(x.astype(bf), WR[l], preferred_element_type=f32) + BF[pl.ds(l, 1), :]
                xs[...] = X0[rows, :].astype(f32) * y + x
                return c2
            lax.fori_loop(0, L, layer_body, 0)
            OUT[rows, :] = xs[...].astype(bf)
            cp = pltpu.make_async_copy(OUT.at[rows], out_hbm.at[rows], sems.at[0])
            cp.start()
            cp.wait()
            return c
        lax.fori_loop(0, B // tf, tile_body, 0)


@jax.jit
def pallas_standalone__dcn_v2_cross__recsys_kernel(
    x0: jax.Array,
    ws: jax.Array,
    bs: jax.Array,
):
    B, D = x0.shape
    L = ws.shape[0]
    tm, R, h1 = 1024, 320, 448
    q = D // 4
    nt = B // tm
    r = tm // 4
    assert B % tm == 0 and nt == 4 and D == 1024 and L % 2 == 0 and L >= 4
    assert (B - R - h1) % (64 * nt) == 0
    return pl.pallas_call(
        functools.partial(_kernel, B=B, D=D, L=L, tm=tm, R=R, h1=h1),
        in_specs=[pl.BlockSpec(memory_space=pl.ANY)] * 3,
        out_specs=pl.BlockSpec(memory_space=pl.ANY),
        out_shape=jax.ShapeDtypeStruct((B, D), x0.dtype),
        scratch_shapes=[
            pltpu.VMEM((B, D), bf),
            pltpu.VMEM((B, D), f32),
            pltpu.VMEM((B, D), f32),
            pltpu.VMEM((L, D, D), bf),
            pltpu.VMEM((49, q // 128, q, 128), bf),
            pltpu.VMEM((49, q // 128, q, 128), bf),
            pltpu.VMEM((B, D), bf),
            pltpu.VMEM((L, D), bf),
            pltpu.VMEM((L, D), f32),
            pltpu.VMEM((6, r, q), f32),
            pltpu.VMEM((6, 4, r, q), f32),
            pltpu.VMEM((L, 8, D), f32),
            pltpu.VMEM((L, 8, 128), f32),
            pltpu.VMEM((L, 8, 128), f32),
            pltpu.SMEM((1,), jnp.int32),
            pltpu.SemaphoreType.DMA((4,)),
        ],
        compiler_params=pltpu.CompilerParams(
            vmem_limit_bytes=120 * 1024 * 1024,
        ),
    )(x0, ws, bs)
```
